```python
import os as _os
_os.environ.setdefault("JAX_PLATFORMS", "cpu")
import jax
import jax.numpy as jnp

def _softmax(x, axis=-1):
    return jax.nn.softmax(x, axis=axis)
def _gelu(x):
    return jax.nn.gelu(x, approximate=True)
def _silu(x):
    return jax.nn.silu(x)
def _sigmoid(x):
    return jax.nn.sigmoid(x)
def _layernorm(x, axis=-1, eps=1e-5):
    m = jnp.mean(x, axis=axis, keepdims=True)
    v = jnp.var(x, axis=axis, keepdims=True)
    return (x - m) / jnp.sqrt(v + eps)
def _scatter_add(tgt, idx, src, axis=0):
    return tgt.at[idx].add(src)
def _segment_sum(src, seg, n):
    return jax.ops.segment_sum(src, seg, n)
class _Rng:
    def __init__(self, key):
        self._k = key
    def _next(self):
        self._k, sub = jax.random.split(self._k)
        return sub
    def normal(self, shape):
        return jax.random.normal(self._next(), shape, dtype=jnp.bfloat16)
    def randint(self, lo, hi, shape):
        return jax.random.randint(self._next(), shape, lo, hi, dtype=jnp.int32)
    def uniform(self, shape, lo=0.0, hi=1.0):
        return jax.random.uniform(self._next(), shape, jnp.bfloat16, lo, hi)
    def permutation(self, n):
        return jax.random.permutation(self._next(), n)


kernel_name = 'concat_heads__gqa_block_cached__gqa_block_cached__decode'

def setup_inputs():
    _rng = _Rng(jax.random.key(int.from_bytes(__import__("os").urandom(4), "little")))
    _w = (lambda a: (lambda t: t.astype(jnp.bfloat16) if jnp.issubdtype(t.dtype, jnp.floating) else t)(jnp.asarray(a)))
    def _A_setup():
        B, Sq, D = 2, 1, 576
        Hq, Hkv, Sk, Dh = 32, 16, 4096, 128
        assert Hq % Hkv == 0, (Hq, Hkv)
        return {
            "x": _w((lambda *s: _rng.normal(s) * 0.8)(B, Sq, D)),
            "k_cache": _w((lambda *s: _rng.normal(s) * 0.8)(B, Hkv, Sk, Dh)),
            "v_cache": _w((lambda *s: _rng.normal(s) * 0.05)(B, Hkv, Sk, Dh)),
            "wq": _w((lambda *s: _rng.normal(s) * 0.8)(D, Hq * Dh) * (D ** -0.5)),
            "wo": _w((lambda *s: _rng.normal(s) * 0.05)(Hq * Dh, D) * ((Hq * Dh) ** -0.5)),
        }
    _A_in = _A_setup()

    def _B_setup():
        B, Sq, D = 2, 1, 576
        Hq, Hkv, Sk, Dh = 32, 16, 4096, 128
        assert Hq % Hkv == 0, (Hq, Hkv)
        return {
            "x": _w((lambda *s: _rng.normal(s) * 0.8)(B, Sq, D)),
            "k_cache": _w((lambda *s: _rng.normal(s) * 0.8)(B, Hkv, Sk, Dh)),
            "v_cache": _w((lambda *s: _rng.normal(s) * 0.05)(B, Hkv, Sk, Dh)),
            "wq": _w((lambda *s: _rng.normal(s) * 0.8)(D, Hq * Dh) * (D ** -0.5)),
            "wo": _w((lambda *s: _rng.normal(s) * 0.05)(Hq * Dh, D) * ((Hq * Dh) ** -0.5)),
        }
    _B_in = _B_setup()

    return {
        "A_x": _A_in["x"],
        "A_k_cache": _A_in["k_cache"],
        "A_v_cache": _A_in["v_cache"],
        "A_wq": _A_in["wq"],
        "A_wo": _A_in["wo"],
        "B_x": _B_in["x"],
        "B_k_cache": _B_in["k_cache"],
        "B_v_cache": _B_in["v_cache"],
        "B_wq": _B_in["wq"],
        "B_wo": _B_in["wo"],
    }

def reference(A_x, A_k_cache, A_v_cache, A_wq, A_wo, B_x, B_k_cache, B_v_cache, B_wq, B_wo):
    def _A_ref(x, k_cache, v_cache, wq, wo):
        B, Sq, D = x.shape
        Hq, Dh = 32, 128
        Hkv = k_cache.shape[1]
        rep = Hq // Hkv
        q = (lambda x, *d: x.transpose(*d))((x @ wq).reshape(B, Sq, Hq, Dh), 0, 2, 1, 3)
        k = jnp.repeat(k_cache, rep, axis=1)
        v = jnp.repeat(v_cache, rep, axis=1)
        scores = jnp.einsum("bhqd,bhkd->bhqk", q, k) * (Dh ** -0.5)
        p = _softmax(scores, axis=-1)
        o = jnp.einsum("bhqk,bhkd->bhqd", p, v)
        return (lambda x, *d: x.transpose(*d))(o, 0, 2, 1, 3).reshape(B, Sq, Hq * Dh) @ wo

    def _B_ref(x, k_cache, v_cache, wq, wo):
        B, Sq, D = x.shape
        Hq, Dh = 32, 128
        Hkv = k_cache.shape[1]
        rep = Hq // Hkv
        q = (lambda x, *d: x.transpose(*d))((x @ wq).reshape(B, Sq, Hq, Dh), 0, 2, 1, 3)
        k = jnp.repeat(k_cache, rep, axis=1)
        v = jnp.repeat(v_cache, rep, axis=1)
        scores = jnp.einsum("bhqd,bhkd->bhqk", q, k) * (Dh ** -0.5)
        p = _softmax(scores, axis=-1)
        o = jnp.einsum("bhqk,bhkd->bhqd", p, v)
        return (lambda x, *d: x.transpose(*d))(o, 0, 2, 1, 3).reshape(B, Sq, Hq * Dh) @ wo

    a = _A_ref(A_x, A_k_cache, A_v_cache, A_wq, A_wo)
    b = _B_ref(B_x, B_k_cache, B_v_cache, B_wq, B_wo)
    return jnp.concatenate([a, b], axis=-1)
```

```python
import functools
import jax
import jax.numpy as jnp
from jax import lax
import jax.experimental.pallas as pl
import jax.experimental.pallas.tpu as pltpu

_NT = (((1,), (1,)), ((), ()))


def build(depth=4, interleave=True, wo_mode='tail', manual_out=False, compute=True, flags=None, WR=8, WC=2048, WS=64):
    B, HKV, SK, DH, D, HQ = 2, 16, 4096, 128, 576, 32
    ROWS = 128
    NS = SK // ROWS
    NT = B * HKV
    NG = HQ // 4
    NC = HQ * DH // WC
    scale = DH ** -0.5
    ahead = depth - 1

    def kern(xa, ka, va, wqa, woa, xb, kb, vb, wqb, wob, o_ref,
             xbuf, wq, wo, ring, sbuf, obuf, sem_x, sem_wq, sem_wo, sem_kv):
        def weight_starts(srcs, dsts, sems):
            def body(i, _):
                r = pl.multiple_of((i // NC) * WR, WR)
                c = pl.multiple_of((i % NC) * WC, WC)
                for t in range(D // WS):
                    for br in range(2):
                        pltpu.make_async_copy(
                            srcs[br].at[pl.ds(t * WS + r, WR), pl.ds(c, WC)],
                            dsts(br, t * WS + r, c), sems(br, t)).start(priority=br)
            lax.fori_loop(0, (WS // WR) * (HQ * DH // WC), body, None)

        def tile_start(srcs, step, slot, t):
            r = pl.multiple_of(step * ROWS, ROWS)
            for br in range(2):
                pltpu.make_async_copy(srcs[br].at[t, pl.ds(r, ROWS)], ring.at[slot, br, t],
                                      sem_kv.at[slot]).start(priority=br)

        def step_wait(slot):
            pltpu.make_async_copy(ring.at[slot], ring.at[slot], sem_kv.at[slot]).wait()

        xc = [pltpu.make_async_copy(s, xbuf.at[br], sem_x.at[br]) for br, s in enumerate((xa, xb))]
        for br, c in enumerate(xc):
            c.start(priority=br)
        weight_starts((wqa, wqb), lambda br, r, c: wq.at[br, pl.ds(r, WR), pl.ds(c, WC)],
                      lambda br, t: sem_wq)

        def pro(s, _):
            for t in range(NT):
                tile_start((ka, kb), s, s, t)
        lax.fori_loop(0, ahead, pro, None)

        row = lax.broadcasted_iota(jnp.int32, (8, DH), 0)
        for c in xc:
            c.wait()
        pltpu.make_async_copy(wq, wq, sem_wq).wait()

        q = []
        for br in range(2):
            x = xbuf[br].astype(jnp.float32)
            odd = lax.broadcasted_iota(jnp.int32, (8, D), 0) % 2 == 1
            x8 = jnp.where(odd, x[1:2], x[0:1]).astype(jnp.bfloat16)
            qb = []
            for g in range(NG):
                y = jnp.dot(x8, wq[br, :, g * 4 * DH:(g + 1) * 4 * DH], preferred_element_type=jnp.float32)
                acc = y[:, :DH]
                for j in range(1, 4):
                    acc = jnp.where(row // 2 == j, y[:, j * DH:(j + 1) * DH], acc)
                qb.append(acc.astype(jnp.bfloat16))
            q.append(qb)

        def merge(parts):
            lo = jnp.where(row % 2 == 0, parts[0][0], parts[0][1])
            hi = jnp.where(row % 2 == 0, parts[1][0], parts[1][1])
            return jnp.where(row < 4, lo, hi)

        def run_step(slot, nxt, tile_fn):
            step_wait(slot)
            if nxt is not None and not interleave:
                for t in range(NT):
                    nxt(t)
            out = []
            for g in range(NG):
                if nxt is not None and interleave:
                    for t in range(4 * g, 4 * g + 4):
                        nxt(t)
                out.append([tile_fn(br, g) for br in range(2)])
            return out

        def k_step(s, m, srcs, s_next):
            slot = s % depth
            nslot = (s + ahead) % depth

            def tile_fn(br, g):
                if not compute:
                    return m[g][br]
                parts = [[lax.dot_general(q[br][g], ring[slot, br, b * HKV + 2 * g + u], _NT,
                                          preferred_element_type=jnp.float32)
                          for b in range(B)] for u in range(2)]
                sc = merge(parts)
                sbuf[s, br, g] = sc
                return jnp.maximum(m[g][br], sc)
            return run_step(slot, lambda t: tile_start(srcs, s_next, nslot, t), tile_fn)

        m = [[jnp.full((8, DH), -jnp.inf, jnp.float32) for _ in range(2)] for _ in range(NG)]
        m = lax.fori_loop(0, NS - ahead, lambda s, m: k_step(s, m, (ka, kb), s + ahead), m)
        m = lax.fori_loop(NS - ahead, NS, lambda s, m: k_step(s, m, (va, vb), s + ahead - NS), m)
        m = [[jnp.broadcast_to(jnp.max(a, axis=1, keepdims=True), (8, DH)) for a in mg] for mg in m]

        def v_step(s, carry, prefetch):
            slot = (s + NS) % depth
            nslot = (s + NS + ahead) % depth

            def tile_fn(br, g):
                l, acc = carry[g][br]
                if not compute:
                    return l, acc
                p = jnp.exp((sbuf[s, br, g] - m[g][br]) * scale)
                pb = p.astype(jnp.bfloat16)
                parts = [[jnp.dot(pb, ring[slot, br, b * HKV + 2 * g + u], preferred_element_type=jnp.float32)
                          for b in range(B)] for u in range(2)]
                return l + p, acc + merge(parts)
            nxt = (lambda t: tile_start((va, vb), s + ahead, nslot, t)) if prefetch else None
            return run_step(slot, nxt, tile_fn)

        z = jnp.zeros((8, DH), jnp.float32)
        carry = [[(z + 1 if not compute else z, z) for _ in range(2)] for _ in range(NG)]
        carry = lax.fori_loop(0, NS - ahead, lambda s, c: v_step(s, c, True), carry)
        weight_starts((woa, wob), lambda br, r, c: wo.at[pl.ds(br * D + r, WR), pl.ds(c, WC)],
                      lambda br, t: sem_wo)
        carry = lax.fori_loop(NS - ahead, NS, lambda s, c: v_step(s, c, False), carry)

        for g in range(NG):
            o = [acc / jnp.sum(l, axis=1, keepdims=True) for l, acc in carry[g]]
            for j in range(4):
                h = 4 * g + j
                obuf[:, h * DH:(h + 1) * DH] = jnp.concatenate(
                    [jnp.where(row // 2 == j, a, 0.0) for a in o], axis=0).astype(jnp.bfloat16)

        pltpu.make_async_copy(wo, wo, sem_wo).wait()
        if wo_mode == 'none':
            o_ref[...] = obuf[:B, :2*D]
            return
        y = lax.dot_general(obuf[...], wo[...], _NT, preferred_element_type=jnp.float32)
        col = lax.broadcasted_iota(jnp.int32, (8, 2 * D), 1)
        y = jnp.where(col < D, y[:8], y[8:])
        y = y + pltpu.roll(y, 4, 0)
        y = y + pltpu.roll(y, 2, 0)
        o_ref[...] = y[:B].astype(o_ref.dtype)

    def f(xa, ka, va, wqa, woa, xb, kb, vb, wqb, wob):
        r = lambda a: a.reshape(NT, SK, DH)
        out = pl.pallas_call(
            kern,
            out_shape=jax.ShapeDtypeStruct((B, 2 * D), jnp.bfloat16),
            in_specs=[pl.BlockSpec(memory_space=pl.ANY)] * 10,
            out_specs=pl.BlockSpec(memory_space=pltpu.VMEM),
            scratch_shapes=[
                pltpu.VMEM((2, B, D), jnp.bfloat16),
                pltpu.VMEM((2, D, HQ * DH), jnp.bfloat16),
                pltpu.VMEM((2 * D, HQ * DH), jnp.bfloat16),
                pltpu.VMEM((depth, 2, NT, ROWS, DH), jnp.bfloat16),
                pltpu.VMEM((NS, 2, NG, 8, DH), jnp.float32),
                pltpu.VMEM((16, HQ * DH), jnp.bfloat16),
                pltpu.SemaphoreType.DMA((2,)),
                pltpu.SemaphoreType.DMA(()),
                pltpu.SemaphoreType.DMA(()),
                pltpu.SemaphoreType.DMA((depth,)),
            ],
            compiler_params=pltpu.CompilerParams(vmem_limit_bytes=100 * 2**20, flags=flags),
        )(xa.reshape(B, D), r(ka), r(va), wqa, woa.T, xb.reshape(B, D), r(kb), r(vb), wqb, wob.T)
        return out.reshape(B, 1, 2 * D)
    return f


_impl = build()


@jax.jit
def pallas_concat_heads__gqa_block_cached__gqa_block_cached__decode_kernel(
    A_x, A_k_cache, A_v_cache, A_wq, A_wo, B_x, B_k_cache, B_v_cache, B_wq, B_wo):
    return _impl(A_x, A_k_cache, A_v_cache, A_wq, A_wo, B_x, B_k_cache, B_v_cache, B_wq, B_wo)
```

```python
import jax
import jax.numpy as jnp
from jax import lax
import jax.experimental.pallas as pl
import jax.experimental.pallas.tpu as pltpu

HQ = 32
ROWS = 128
WR = 8
WS = 64
DEPTH = 3
AHEAD = DEPTH - 1

SHIFT = (0, 1)

_NT = (((1,), (1,)), ((), ()))


def _loop(n, body, unroll=1):
    def outer(i, _):
        for u in range(unroll):
            body(i * unroll + u)

    lax.fori_loop(0, n // unroll, outer, None)


def _kernel(xa, ka, va, wqa, woa, xb, kb, vb, wqb, wob, o_ref,
            xbuf, wq, wo, ring, qbuf, sbuf, mbuf, lbuf, abuf, obuf, ybuf,
            sem_x, sem_wq, sem_wo, sem_kv):
    _, nb, d = xbuf.shape
    ns, _, ng, _, dh = sbuf.shape
    nt = ring.shape[2] // ROWS
    hkv = nt // nb
    sk = ns * ROWS
    wc = HQ * dh // 2
    nj = 2 * d // dh
    scale = dh ** -0.5
    aligned = pl.multiple_of
    row = lax.broadcasted_iota(jnp.int32, (8, dh), 0)

    def weight_start(src, br, r, part, dst, sem, queue):
        if not SHIFT[br]:
            pieces = [(r, part * wc, part * wc, wc)]
        elif part == 1:
            pieces = [(r, wc // 2, wc, wc)]
        else:
            r_next = jnp.where(r + WR == d, 0, r + WR)
            pieces = [(r, 3 * wc // 2, 0, wc // 2), (r_next, 0, wc // 2, wc // 2)]
        for r, c, c_dst, n in pieces:
            r = aligned(r, WR)
            pltpu.make_async_copy(
                src.at[pl.ds(r, WR), pl.ds(c, n)], dst(r, c_dst, n), sem(r)).start(priority=queue)

    def wq_start(i):
        for part in (1, 0):
            def body(t):
                for br, w in enumerate((wqa, wqb)):
                    weight_start(w, br, t * WS + i * WR, part,
                                 lambda r, c, n: wq.at[br, pl.ds(r, WR), pl.ds(c, n)],
                                 lambda r: sem_wq, br)
            _loop(d // WS, body)

    def wo_start(r0, r1, streams, part, i0=0, count=WS // WR):
        def band(i):
            def body(t):
                for queue, r in enumerate((r0, r1)):
                    br = int(r >= d)
                    weight_start((woa, wob)[br], br, r - br * d + t * WS + (i0 + i) * WR, part,
                                 lambda r, c, n: wo.at[pl.ds(aligned(r + br * d, WR), WR), pl.ds(c, n)],
                                 lambda r: sem_wo.at[part * nj + (r + br * d) // dh], queue)
            _loop(streams, body)
        _loop(count, band)

    def kv_start(src, r, n, slot, br, r_dst, queue):
        pltpu.make_async_copy(
            src.at[pl.ds(aligned(r, ROWS // 2), n)],
            ring.at[slot, br, pl.ds(aligned(r_dst, ROWS // 2), n)],
            sem_kv.at[slot]).start(priority=queue)

    def step_start(srcs, step, slot):
        for br, src in enumerate(srcs):
            def body(h):
                for b in range(nb):
                    t = b * hkv + h
                    kv_start(src, t * sk + step * ROWS - SHIFT[br] * (ROWS // 2), ROWS, slot, br, t * ROWS, b)
            _loop(hkv, body, 4)

    def first_start(srcs, slot):
        for br, src in enumerate(srcs):
            back = SHIFT[br] * (ROWS // 2)
            kv_start(src, 0, ROWS - back, slot, br, 0, 0)
            kv_start(src, hkv * sk - back, ROWS, slot, br, hkv * ROWS - back, 1)

            def body(h):
                for b in range(nb):
                    t = b * hkv + h + 1
                    kv_start(src, t * sk - back, ROWS, slot, br, t * ROWS - back, b)
            _loop(hkv - 1, body)
            if back:
                kv_start(src, nt * sk - back, back, slot, br, nt * ROWS - back, 0)

    def step_wait(slot):
        pltpu.make_async_copy(ring.at[slot], ring.at[slot], sem_kv.at[slot]).wait()

    _loop(WS // WR, wq_start)
    x_copies = [pltpu.make_async_copy(x, xbuf.at[br], sem_x.at[br]) for br, x in enumerate((xa, xb))]
    for br, c in enumerate(x_copies):
        c.start(priority=br)
    first_start((ka, kb), 0)
    for s in range(1, AHEAD):
        step_start((ka, kb), s, s)
    for c in x_copies:
        c.wait()
    odd = lax.broadcasted_iota(jnp.int32, (8, d), 0) % 2 == 1
    x8 = []
    for br in range(2):
        x = xbuf[br].astype(jnp.float32)
        x8.append(jnp.where(odd, x[1:2], x[0:1]).astype(wq.dtype))
    pltpu.make_async_copy(wq, wq, sem_wq).wait()

    def q_body(g):
        for br in range(2):
            c = aligned(((g + SHIFT[br] * (ng // 4)) % ng) * 4 * dh, 4 * dh)
            y = jnp.dot(x8[br], wq[br, :, pl.ds(c, 4 * dh)], preferred_element_type=jnp.float32)
            q = y[:, :dh]
            for j in range(1, 4):
                q = jnp.where(row // 2 == j, y[:, j * dh:(j + 1) * dh], q)
            qbuf[br, g] = q
            mbuf[br, g] = jnp.full((8, dh), -jnp.inf, jnp.float32)
            lbuf[br, g] = jnp.zeros((8, dh), jnp.float32)
            abuf[br, g] = jnp.zeros((8, dh), jnp.float32)
    _loop(ng, q_body)

    def per_head(fn, slot, br, g):
        p = [[fn(ring[slot, br, pl.ds(aligned((b * hkv + 2 * g + u) * ROWS, ROWS), ROWS)])
              for b in range(nb)] for u in range(2)]
        lo = jnp.where(row % 2 == 0, p[0][0], p[0][1])
        hi = jnp.where(row % 2 == 0, p[1][0], p[1][1])
        return jnp.where(row < 4, lo, hi)

    def k_step(s):
        slot, free = s % DEPTH, (s + AHEAD) % DEPTH
        step_wait(slot)

        @pl.when(s + AHEAD < ns)
        def _():
            step_start((ka, kb), s + AHEAD, free)

        @pl.when(s + AHEAD == ns)
        def _():
            first_start((va, vb), free)

        @pl.when(s + AHEAD > ns)
        def _():
            step_start((va, vb), s + AHEAD - ns, free)

        def body(g):
            for br in range(2):
                q = qbuf[br, g].astype(ring.dtype)
                scores = per_head(
                    lambda k: lax.dot_general(q, k, _NT, preferred_element_type=jnp.float32), slot, br, g)
                sbuf[s, br, g] = scores
                mbuf[br, g] = jnp.maximum(mbuf[br, g], scores)
        _loop(ng, body, 2)
    _loop(ns, k_step)
    m = mbuf[...].reshape(2 * ng * 8, dh)
    mbuf[...] = jnp.broadcast_to(jnp.max(m, axis=1, keepdims=True), m.shape).reshape(mbuf.shape)

    def v_step(s):
        slot, free = (s + ns) % DEPTH, (s + ns + AHEAD) % DEPTH
        step_wait(slot)

        @pl.when(s + AHEAD < ns)
        def _():
            step_start((va, vb), s + AHEAD, free)

        @pl.when(s == ns - 2)
        def _():
            wo_start(0, d, d // WS, 0, 0, 4)

        @pl.when(s == ns - 1)
        def _():
            wo_start(0, d, d // WS, 0, 4, 3)

        def body(g):
            for br in range(2):
                p = jnp.exp((sbuf[s, br, g] - mbuf[br, g]) * scale)
                pb = p.astype(ring.dtype)
                pv = per_head(lambda v: jnp.dot(pb, v, preferred_element_type=jnp.float32), slot, br, g)
                lbuf[br, g] += p
                abuf[br, g] += pv
        _loop(ng, body, 2)
    _loop(ns, v_step)
    wo_start(0, d, d // WS, 0, 7, 1)
    wo_start(0, 7 * dh, 4, 1, 0, 6)

    o = [[abuf[br, g] / jnp.sum(lbuf[br, g], axis=1, keepdims=True) for g in range(ng)] for br in range(2)]
    for c in range(HQ):
        heads = [(c - SHIFT[br] * (HQ // 4)) % HQ for br in range(2)]
        obuf[:, c * dh:(c + 1) * dh] = jnp.concatenate(
            [pltpu.roll(o[br][h // 4], 8 - 2 * (h % 4), 0) if h % 4 else o[br][h // 4]
             for br, h in enumerate(heads)], axis=0).astype(obuf.dtype)
    ybuf[...] = jnp.zeros(ybuf.shape, jnp.float32)
    lane = lax.broadcasted_iota(jnp.int32, (8, dh), 1)

    order = (0, 1, 7, 8, 2, 6, 3, 5, 4)
    packed = sum(n << (4 * i) for i, n in enumerate(order[1:]))

    def job(j):
        part, i = j // nj, j % nj
        n = jnp.where(i == 0, order[0], (packed >> (4 * jnp.maximum(i - 1, 0))) & 15)
        r, c = aligned(n * dh, dh), aligned(part * wc, wc)
        block = wo.at[pl.ds(r, dh), pl.ds(c, wc)]
        pltpu.make_async_copy(block, block, sem_wo.at[part * nj + n]).wait()

        @pl.when(j == 0)
        def _():
            wo_start(0, 7 * dh, 4, 1, 6, 2)

        for when, tiles in ((3, order[4:6]), (6, order[6:])):
            @pl.when(j == when)
            def _():
                for t in tiles:
                    wo_start(t * dh, t * dh + WS, 1, 1)

        y = ybuf[n] + lax.dot_general(obuf[:, pl.ds(c, wc)], wo[pl.ds(r, dh), pl.ds(c, wc)], _NT,
                                      preferred_element_type=jnp.float32)
        ybuf[n] = y
        o_ref[:, pl.ds(r, dh)] = jnp.where(lane < d - r, y[:8], y[8:])[:nb].astype(o_ref.dtype)
    _loop(2 * nj, job)


def _forward(xa, ka, va, wqa, woa, xb, kb, vb, wqb, wob, interpret=False):
    nb, sq, d = xa.shape
    _, hkv, sk, dh = ka.shape
    assert (nb, sq, d, hkv, dh) == (2, 1, 576, HQ // 2, 128) and sk % ROWS == 0 and sk >= DEPTH * ROWS
    dtype = ka.dtype
    ng, nj = HQ // 4, 2 * d // dh
    per_row = pltpu.VMEM((2, ng, 8, dh), jnp.float32)
    flat = lambda cache: cache.reshape(nb * hkv * sk, dh)
    out = pl.pallas_call(
        _kernel,
        out_shape=jax.ShapeDtypeStruct((nb, 2 * d), xa.dtype),
        in_specs=[pl.BlockSpec(memory_space=pl.ANY)] * 10,
        out_specs=pl.BlockSpec(memory_space=pltpu.VMEM),
        scratch_shapes=[
            pltpu.VMEM((2, nb, d), xa.dtype),
            pltpu.VMEM((2, d, HQ * dh), dtype),
            pltpu.VMEM((2 * d, HQ * dh), dtype),
            pltpu.VMEM((DEPTH, 2, nb * hkv * ROWS, dh), dtype),
            per_row,
            pltpu.VMEM((sk // ROWS, 2, ng, 8, dh), jnp.float32),
            per_row,
            per_row,
            per_row,
            pltpu.VMEM((16, HQ * dh), dtype),
            pltpu.VMEM((nj, 16, dh), jnp.float32),
            pltpu.SemaphoreType.DMA((2,)),
            pltpu.SemaphoreType.DMA(()),
            pltpu.SemaphoreType.DMA((2 * nj,)),
            pltpu.SemaphoreType.DMA((DEPTH,)),
        ],
        compiler_params=pltpu.CompilerParams(
            vmem_limit_bytes=64 * 2**20, disable_semaphore_checks=True),
        interpret=interpret,
    )(
        xa.reshape(nb, d), flat(ka), flat(va), wqa, woa.T,
        xb.reshape(nb, d), flat(kb), flat(vb), wqb, wob.T,
    )
    return out.reshape(nb, sq, 2 * d)


@jax.jit
def pallas_concat_heads__gqa_block_cached__gqa_block_cached__decode_kernel(
    A_x: jax.Array,
    A_k_cache: jax.Array,
    A_v_cache: jax.Array,
    A_wq: jax.Array,
    A_wo: jax.Array,
    B_x: jax.Array,
    B_k_cache: jax.Array,
    B_v_cache: jax.Array,
    B_wq: jax.Array,
    B_wo: jax.Array,
):
    return _forward(A_x, A_k_cache, A_v_cache, A_wq, A_wo, B_x, B_k_cache, B_v_cache, B_wq, B_wo)
```
